```python
import os as _os
_os.environ.setdefault("JAX_PLATFORMS", "cpu")
import jax
import jax.numpy as jnp

def _softmax(x, axis=-1):
    return jax.nn.softmax(x, axis=axis)
def _gelu(x):
    return jax.nn.gelu(x, approximate=True)
def _silu(x):
    return jax.nn.silu(x)
def _sigmoid(x):
    return jax.nn.sigmoid(x)
def _layernorm(x, axis=-1, eps=1e-5):
    m = jnp.mean(x, axis=axis, keepdims=True)
    v = jnp.var(x, axis=axis, keepdims=True)
    return (x - m) / jnp.sqrt(v + eps)
def _scatter_add(tgt, idx, src, axis=0):
    return tgt.at[idx].add(src)
def _segment_sum(src, seg, n):
    return jax.ops.segment_sum(src, seg, n)
class _Rng:
    def __init__(self, key):
        self._k = key
    def _next(self):
        self._k, sub = jax.random.split(self._k)
        return sub
    def normal(self, shape):
        return jax.random.normal(self._next(), shape, dtype=jnp.bfloat16)
    def randint(self, lo, hi, shape):
        return jax.random.randint(self._next(), shape, lo, hi, dtype=jnp.int32)
    def uniform(self, shape, lo=0.0, hi=1.0):
        return jax.random.uniform(self._next(), shape, jnp.bfloat16, lo, hi)
    def permutation(self, n):
        return jax.random.permutation(self._next(), n)


kernel_name = 'parallel_sum__mha_block__swiglu_ffn__prompt'

def setup_inputs():
    _rng = _Rng(jax.random.key(int.from_bytes(__import__("os").urandom(4), "little")))
    _w = (lambda a: (lambda t: t.astype(jnp.bfloat16) if jnp.issubdtype(t.dtype, jnp.floating) else t)(jnp.asarray(a)))
    def _A_setup():
        B, S, D, H = 1, 2048, 640, 32
        return {
            "x": _w((lambda *s: _rng.normal(s) * 0.05)(B, S, D)),
            "wqkv": _w((lambda *s: _rng.normal(s) * 0.1)(D, 3 * D)),
            "wo": _w((lambda *s: _rng.normal(s) * 0.05)(D, D)),
        }
    _A_in = _A_setup()

    def _B_setup():
        B, S, D, F = 1, 2048, 640, 1536
        return {
            "x": _w((lambda *s: _rng.normal(s) * 0.05)(B, S, D)),
            "w_gate": _w((lambda *s: _rng.normal(s) * 0.05)(D, F)),
            "w_up": _w((lambda *s: _rng.normal(s) * 0.05)(D, F)),
            "w_down": _w((lambda *s: _rng.normal(s) * 0.05)(F, D)),
        }
    _B_in = _B_setup()

    return {
        "A_x": _A_in["x"],
        "A_wqkv": _A_in["wqkv"],
        "A_wo": _A_in["wo"],
        "B_x": _B_in["x"],
        "B_w_gate": _B_in["w_gate"],
        "B_w_up": _B_in["w_up"],
        "B_w_down": _B_in["w_down"],
    }

def reference(A_x, A_wqkv, A_wo, B_x, B_w_gate, B_w_up, B_w_down):
    def _A_ref(x, wqkv, wo):
        B, S, D = x.shape
        H = 32
        Dh = D // H
        qkv = (lambda x, *d: x.transpose(*d))((x @ wqkv).reshape(B, S, 3, H, Dh), 2, 0, 3, 1, 4)
        q, k, v = qkv[0], qkv[1], qkv[2]
        scores = jnp.einsum("bhqd,bhkd->bhqk", q, k) * (Dh ** -0.5)
        p = _softmax(scores, axis=-1)
        o = jnp.einsum("bhqk,bhkd->bhqd", p, v)
        return (lambda x, *d: x.transpose(*d))(o, 0, 2, 1, 3).reshape(B, S, D) @ wo

    def _B_ref(x, w_gate, w_up, w_down):
        g = _silu(x @ w_gate)
        u = x @ w_up
        return (g * u) @ w_down

    x = A_x
    xn = _layernorm(x, axis=-1)
    return x + _A_ref(xn, A_wqkv, A_wo) + _B_ref(xn, B_w_gate, B_w_up, B_w_down)
```

```python
import math

import jax
import jax.numpy as jnp
from jax import lax
import jax.experimental.pallas as pl
import jax.experimental.pallas.tpu as pltpu

_H = 32
_EPS = 1e-5
_BQ = 512
_CK = 128
_RC = 512
_VR = 24

_F32 = jnp.float32
_BF16 = jnp.bfloat16


def _mm(a, b):
    return lax.dot_general(a, b, (((1,), (0,)), ((), ())), preferred_element_type=_F32)


def _mm_nt(a, b):
    return lax.dot_general(a, b, (((1,), (1,)), ((), ())), preferred_element_type=_F32)


def _kernel(
    x_hbm, wqkv_hbm, wo_hbm, wg_hbm, wu_hbm, wd_hbm,
    out_hbm,
    x_v, xn_v, wqkv_v, wo_v, wg_v, wu_v, wd_v, wqvt_v,
    qt_v, kw_v, vt_v, ot_v, s_v, out_v,
    x_sem, w_sem, o_sem,
):
    S, D = x_v.shape
    dh = D // _H
    n_rc = S // _RC
    n_q = S // _BQ
    n_ck = S // _CK

    def rows(i):
        return pl.ds(i * _RC, _RC)

    x_cp = [
        pltpu.make_async_copy(x_hbm.at[rows(i)], x_v.at[rows(i)], x_sem.at[i])
        for i in range(n_rc)
    ]
    w_cp = [
        pltpu.make_async_copy(src, dst, w_sem.at[i])
        for i, (src, dst) in enumerate(
            [(wqkv_hbm, wqkv_v), (wg_hbm, wg_v), (wu_hbm, wu_v), (wd_hbm, wd_v), (wo_hbm, wo_v)]
        )
    ]
    x_cp[0].start()
    w_cp[0].start()
    for cp in x_cp[1:] + w_cp[1:]:
        cp.start()

    w_cp[0].wait()
    wqvt_v[0:D, :] = wqkv_v[:, 0:D].T
    wqvt_v[D:2 * D, :] = wqkv_v[:, 2 * D:3 * D].T
    qt_v[D:, :] = jnp.zeros((qt_v.shape[0] - D, S), _BF16)

    q_scale = (dh ** -0.5) * math.log2(math.e)
    lane = lax.broadcasted_iota(jnp.int32, (_RC, 128), 1)
    for i in range(n_rc):
        x_cp[i].wait()
        x = x_v[rows(i), :].astype(_F32)
        xc = x - jnp.mean(x, axis=-1, keepdims=True)
        var = jnp.mean(xc * xc, axis=-1, keepdims=True)
        xn = (xc * lax.rsqrt(var + _EPS)).astype(_BF16)
        xn_v[rows(i), :] = xn
        k = _mm(xn, wqkv_v[:, D:2 * D])
        nt = D // 128
        for t in range(nt):
            lo = k[:, 128 * t:128 * (t + 1)]
            kw_v[2 * t, rows(i), :] = lo.astype(_BF16)
            t1 = min(t + 1, nt - 1)
            hi = k[:, 128 * t1:128 * (t1 + 1)]
            kw_v[2 * t + 1, rows(i), :] = jnp.where(lane >= 64, lo, hi).astype(_BF16)
        qt_v[0:D, rows(i)] = (_mm_nt(wqvt_v[0:D, :], xn) * q_scale).astype(_BF16)
        vt_v[:, rows(i)] = _mm_nt(wqvt_v[D:2 * D, :], xn)

    def q_tile(h, qb):
        j = (h * dh) // 64
        odd = j % 2
        top = pl.multiple_of(64 * (j + odd), 64)
        bot = pl.multiple_of(64 * (j + 1 - odd), 64)
        cols = slice(qb * _BQ, (qb + 1) * _BQ)
        r = lax.broadcasted_iota(jnp.int32, (64, _BQ), 0)
        halves = []
        for base in (top, bot):
            rel = r + (base - h * dh)
            keep = jnp.logical_and(rel >= 0, rel < dh)
            q = qt_v[pl.ds(base, 64), cols].astype(_F32)
            halves.append(jnp.where(keep, q, 0.0).astype(_BF16))
        return j, jnp.concatenate(halves, axis=0)

    def attn_step(new, old, m_old):
        if new is not None:
            j, qt = q_tile(*new)
        if old is not None:
            ho, qo = old
            base = pl.multiple_of((ho * dh) // 8 * 8, 8)
            off = ho * dh - base
            ones_row = jnp.where(off == 0, _VR - 1, 0)
            vrow = lax.broadcasted_iota(jnp.int32, (_VR, _CK), 0)
        m_new = None
        acc = None
        for c in range(n_ck):
            ks = slice(c * _CK, (c + 1) * _CK)
            if old is not None:
                s_old = s_v[ks, :]
            if new is not None:
                s_new = _mm(kw_v[j, ks, :], qt)
            if old is not None:
                p = jnp.exp2(s_old - m_old).astype(_BF16)
                vt = jnp.where(vrow == ones_row, 1.0, vt_v[pl.ds(base, _VR), ks])
                pv = _mm(vt, p)
                acc = pv if acc is None else acc + pv
            if new is not None:
                s_v[ks, :] = s_new
                mc = jnp.max(s_new.reshape(_CK // 8, 8, _BQ), axis=0)
                m_new = mc if m_new is None else jnp.maximum(m_new, mc)
        if old is not None:
            den = jnp.where(off == 0, acc[_VR - 1:_VR, :], acc[0:1, :])
            rel = lax.broadcasted_iota(jnp.int32, (_VR, _BQ), 0) - off
            keep = jnp.logical_and(rel >= 0, rel < dh)
            cols = slice(qo * _BQ, (qo + 1) * _BQ)
            win = pl.ds(base, _VR)
            ot_v[win, cols] = jnp.where(keep, acc / den, ot_v[win, cols])
        if new is not None:
            return jnp.max(m_new, axis=0, keepdims=True)
        return None

    ot_v[...] = jnp.zeros(ot_v.shape, _F32)
    m = attn_step((0, 0), None, None)

    def head_body(h, m):
        for qb in range(1, n_q):
            m = attn_step((h, qb), (h, qb - 1), m)
        return attn_step((jnp.minimum(h + 1, _H - 1), 0), (h, n_q - 1), m)

    lax.fori_loop(0, _H, head_body, m)

    for cp in w_cp[1:]:
        cp.wait()
    o_cp = [
        pltpu.make_async_copy(out_v.at[rows(i)], out_hbm.at[rows(i)], o_sem.at[i])
        for i in range(n_rc)
    ]
    for i in range(n_rc):
        xn = xn_v[rows(i), :]
        g = _mm(xn, wg_v[...])
        u = _mm(xn, wu_v[...])
        hid = (g * jax.nn.sigmoid(g) * u).astype(_BF16)
        o = ot_v[:, rows(i)].T.astype(_BF16)
        y = _mm(hid, wd_v[...]) + _mm(o, wo_v[...])
        out_v[rows(i), :] = (x_v[rows(i), :].astype(_F32) + y).astype(out_v.dtype)
        o_cp[i].start()
    for cp in o_cp:
        cp.wait()


@jax.jit
def pallas_parallel_sum__mha_block__swiglu_ffn__prompt_kernel(
    A_x: jax.Array,
    A_wqkv: jax.Array,
    A_wo: jax.Array,
    B_x: jax.Array,
    B_w_gate: jax.Array,
    B_w_up: jax.Array,
    B_w_down: jax.Array,
):
    del B_x
    B, S, D = A_x.shape
    F = B_w_gate.shape[1]
    assert B == 1 and D // _H == 20 and S % _BQ == 0 and S % _RC == 0
    n_rc = S // _RC
    any_spec = pl.BlockSpec(memory_space=pl.ANY)
    out = pl.pallas_call(
        _kernel,
        out_shape=jax.ShapeDtypeStruct((S, D), A_x.dtype),
        in_specs=[any_spec] * 6,
        out_specs=any_spec,
        scratch_shapes=[
            pltpu.VMEM((S, D), A_x.dtype),
            pltpu.VMEM((S, D), _BF16),
            pltpu.VMEM((D, 3 * D), _BF16),
            pltpu.VMEM((D, D), _BF16),
            pltpu.VMEM((D, F), _BF16),
            pltpu.VMEM((D, F), _BF16),
            pltpu.VMEM((F, D), _BF16),
            pltpu.VMEM((2 * D, D), _BF16),
            pltpu.VMEM((D + 64, S), _BF16),
            pltpu.VMEM((2 * (D // 128), S, 128), _BF16),
            pltpu.VMEM((D, S), _F32),
            pltpu.VMEM((D, S), _F32),
            pltpu.VMEM((S, _BQ), _F32),
            pltpu.VMEM((S, D), A_x.dtype),
            pltpu.SemaphoreType.DMA((n_rc,)),
            pltpu.SemaphoreType.DMA((5,)),
            pltpu.SemaphoreType.DMA((n_rc,)),
        ],
        compiler_params=pltpu.CompilerParams(vmem_limit_bytes=100 * 1024 * 1024),
        name="fused_mha_swiglu",
    )(
        A_x.reshape(S, D),
        A_wqkv.astype(_BF16),
        A_wo.astype(_BF16),
        B_w_gate.astype(_BF16),
        B_w_up.astype(_BF16),
        B_w_down.astype(_BF16),
    )
    return out.reshape(B, S, D)
```

```python
import functools
import math

import jax
import jax.numpy as jnp
from jax import lax
import jax.experimental.pallas as pl
import jax.experimental.pallas.tpu as pltpu

_H = 32
_EPS = 1e-5
_BQ = 512
_CK = 128
_LAG = 2
_DP = 24
_NV = 256
_GD = 4
_X_CUT = (0, 128, 256, 512, 896, 1280, 2048)
_O_CUT = (0, 128, 512, 1024, 1536, 1920, 2048)
_LAT, _EXP_SPAN, _LOOKAHEAD, _VPU_RATE = 125, 64, 32, 3.1

_F32 = jnp.float32
_BF16 = jnp.bfloat16
_I32 = jnp.int32


def _mm(a, b):
    return lax.dot_general(a, b, (((1,), (0,)), ((), ())), preferred_element_type=_F32)


def _pack(v):
    return pltpu.bitcast(v, _I32)


def _unpack(v):
    return pltpu.bitcast(v, _BF16)


def _tile(t, n=1):
    return slice(128 * t, 128 * (t + n))


def _per_vreg(v, fn):
    return jnp.concatenate([
        jnp.concatenate([fn(v[r:r + 8, c:c + 128]) for c in range(0, v.shape[1], 128)], axis=1)
        for r in range(0, v.shape[0], 8)], axis=0)


def _mix(*lists):
    keyed = [((j + 0.5) / len(l), n, t) for n, l in enumerate(lists) for j, t in enumerate(l)]
    return [t for _, _, t in sorted(keyed, key=lambda e: e[:2])]


def _kernel(
    x_hbm, wqkv_hbm, wo_hbm, wg_hbm, wu_hbm, wd_hbm,
    out_hbm,
    x_v, xn_v, xnt_v, wq_v, wk_v, wv_v, wo_v, wg_v, wu_v, wd_v, wqt_v, wvt_v,
    kp_v, q_v, k_v, v_v, o_v, sa_v, sb_v, kb0_v, kb1_v, gu_v, hid_v, y_v, out_v, z_v,
    x_sem, w_sem, o_sem,
):
    S, D = x_v.shape
    F = wg_v.shape[1]
    dh = D // _H
    n_q = S // _BQ
    n_ck = S // _CK
    rb = y_v.shape[1]
    bufs = (sa_v, sb_v)
    kbs = (kb0_v, kb1_v)
    partial = functools.partial

    x_cp = [
        pltpu.make_async_copy(x_hbm.at[lo:hi], x_v.at[lo:hi], x_sem.at[i])
        for i, (lo, hi) in enumerate(zip(_X_CUT[:-1], _X_CUT[1:]))
    ]
    w_cp = [
        pltpu.make_async_copy(src, dst, w_sem.at[i])
        for i, (src, dst) in enumerate([
            (wqkv_hbm.at[:, D:2 * D], wk_v),
            (wqkv_hbm.at[:, 0:D], wq_v),
            (wqkv_hbm.at[:, 2 * D:3 * D], wv_v),
            (wg_hbm, wg_v.bitcast(_BF16)),
            (wu_hbm, wu_v.bitcast(_BF16)),
            (wd_hbm, wd_v.bitcast(_BF16)),
            (wo_hbm, wo_v),
        ])
    ]
    o_cp = [
        pltpu.make_async_copy(out_v.at[lo:hi], out_hbm.at[lo:hi], o_sem.at[i])
        for i, (lo, hi) in enumerate(zip(_O_CUT[:-1], _O_CUT[1:]))
    ]

    def now(v):
        return v

    def pacer():
        never = z_v[...] != 0.0
        return lambda anchor: (
            lambda v: jnp.where(never, pltpu.bitcast(anchor, v.dtype), v))

    def layernorm(r0, pace):
        x = _unpack(_per_vreg(_pack(x_v[r0:r0 + 32, :]), pace)).astype(_F32)
        xc = x - jnp.mean(x, axis=-1, keepdims=True)
        var = jnp.mean(xc * xc, axis=-1, keepdims=True)
        xn = (xc * lax.rsqrt(var + _EPS)).astype(_BF16)
        xn_v[r0 // rb, r0 % rb // 2:r0 % rb // 2 + 16, :] = _pack(xn)

    def transpose(src, dst, pace):
        dst[...] = _unpack(_per_vreg(_pack(src[...]), pace)).T

    def spread_k(h, r0, pace):
        t, off = divmod(h * dh, 128)
        w = _per_vreg(kp_v[r0:r0 + 64, _tile(t)], pace)
        if off + dh > 128:
            lane = lax.broadcasted_iota(_I32, w.shape, 1)
            w = jnp.where(lane >= 64, w, kp_v[r0:r0 + 64, _tile(t + 1)])
        k_v[h, r0:r0 + 64, :] = pltpu.roll(w, 128 - off, 1) if off else w

    def splat_keys(h, slot, d0, g, pace):
        kk = _unpack(pace(k_v[h, 8 * g:8 * g + 8, :])).astype(_F32)
        for d in range(d0, d0 + 5):
            kbs[slot][0, d, 16 * g:16 * g + 16, :] = jnp.broadcast_to(kk[:, d:d + 1], (16, 128))

    splats = [(d0, g) for d0 in range(0, dh, 5) for g in range(_NV // 16)]

    def dot_paced(lhs, rhs, tasks, after):
        nk = lhs.shape[1] // 128
        m8 = lhs.shape[0] // 8
        parts = [_mm(lhs[:, _tile(t)], rhs[_tile(t), :]) for t in range(nk)]
        for j, task in enumerate(tasks):
            t, r = divmod(int(j * (nk - 0.4) * m8 / len(tasks)), m8)
            task(after(parts[t][8 * r:8 * r + 8, 0:128]))
        return functools.reduce(jnp.add, parts)

    def project_k(r0, n, tasks, after):
        xn = _unpack(xn_v[r0 // rb:(r0 + n) // rb].reshape(n // 2, D))
        k = jnp.concatenate([
            dot_paced(xn, wk_v[:, 0:512], tasks, after), _mm(xn, wk_v[:, 512:D])], axis=1)
        kp_v[r0 // 2:(r0 + n) // 2, :] = _pack(k.astype(_BF16))

    sub = lax.broadcasted_iota(_I32, (8, _BQ), 0)

    def project_q(i, tasks, after):
        cols = slice(i * _BQ, (i + 1) * _BQ)
        qt = dot_paced(wqt_v[...], xnt_v[:, cols], tasks, after)
        qt = qt * (dh ** -0.5 * math.log2(math.e))
        for h in range(_H):
            base = h * dh // 8 * 8
            q3 = [qt[base + 8 * j:base + 8 * j + 8] for j in range(3)]
            if h % 2 == 0:
                q3[2] = jnp.where(sub < 4, q3[2], 0.0)
            else:
                q3 = [pltpu.roll(t, 4, 0) for t in q3] + [0.0]
                q3 = [jnp.where(sub < 4, q3[j], q3[j + 1]) for j in range(3)]
            q_v[h, :, cols] = jnp.concatenate(q3, axis=0)

    def project_v(i, tasks, after):
        cols = slice(i * _BQ, (i + 1) * _BQ)
        vt = dot_paced(wvt_v[...], xnt_v[:, cols], tasks, after)
        for h in range(_H):
            base = h * dh // 8 * 8
            if h % 2 == 0:
                v_v[h, 0:16, cols] = vt[base:base + 16]
                v_v[h, 16:24, cols] = jnp.where(sub == 7, 1.0, vt[base + 16:base + 24])
            else:
                v_v[h, 0:8, cols] = jnp.where(sub == 0, 1.0, vt[base:base + 8])
                v_v[h, 8:24, cols] = vt[base + 8:base + 24]

    def ln_tasks(lo, hi):
        return [partial(layernorm, r0) for r0 in range(lo, hi, 32)]

    def xt_tasks(lo, hi):
        return [partial(transpose, xn_v.at[j, :, _tile(t)], xnt_v.at[_tile(t), _tile(j)])
                for j in range(lo // rb, hi // rb) for t in range(D // 128)]

    def wt_tasks(src, dst):
        return [partial(transpose, src.at[_tile(r), _tile(c)], dst.at[_tile(c), _tile(r)])
                for r in range(D // 128) for c in range(D // 128)]

    def ks_tasks(lo, hi):
        return [partial(spread_k, h, r0 // 2) for r0 in range(lo, hi, 128) for h in range(_H)]

    for cp in (x_cp[0], x_cp[1], w_cp[0]):
        cp.start()
    sa_v[S - _LAG * _CK:, :] = jnp.zeros((_LAG * _CK, _BQ), _F32)
    sb_v[...] = jnp.zeros(sb_v.shape, _F32)
    o_v[0, :, S - 2 * _BQ:S - _BQ] = jnp.zeros((_DP, _BQ), _F32)
    z_v[...] = jnp.zeros(z_v.shape, _F32)
    x_cp[0].wait()
    x_cp[2].start()
    x_cp[1].wait()
    for task in ln_tasks(0, 256):
        task(now)
    x_cp[2].wait()
    x_cp[3].start()
    x_cp[4].start()
    w_cp[0].wait()
    after = pacer()
    project_k(0, 256, ln_tasks(256, 512), after)
    project_k(256, 128, [], after)
    x_cp[3].wait()
    for cp in (x_cp[5], w_cp[1], w_cp[2]):
        cp.start()
    x_cp[4].wait()
    after = pacer()
    project_k(384, 128, ln_tasks(512, 640), after)
    project_k(512, 128, ln_tasks(640, 896), after)
    project_k(640, 256, ln_tasks(896, 1280), after)
    project_k(896, 128, xt_tasks(0, 256), after)
    w_cp[1].wait()
    w_cp[2].wait()
    for cp in w_cp[3:]:
        cp.start()
    x_cp[5].wait()
    after = pacer()
    project_k(1024, 256, _mix(wt_tasks(wq_v, wqt_v), xt_tasks(256, 512)), after)
    project_q(0, _mix(ln_tasks(1280, 1536), xt_tasks(512, 1024)), after)
    project_k(1280, 256, ln_tasks(1536, 1792), after)
    project_q(1, _mix(ln_tasks(1792, 2048), xt_tasks(1024, 1536)), after)
    project_k(1536, 512, _mix(xt_tasks(1536, 2048), ks_tasks(0, 256)), after)
    project_q(2, _mix(wt_tasks(wv_v, wvt_v), ks_tasks(256, 512)), after)
    project_q(3, ks_tasks(512, 896), after)
    project_v(0, ks_tasks(896, 1280), after)
    project_v(1, ks_tasks(1280, 1664), after)
    project_v(2, ks_tasks(1664, 2048), after)
    project_v(3, [partial(splat_keys, 0, 0, *sp) for sp in splats], after)
    for cp in w_cp[3:]:
        cp.wait()

    def pv_chunk(h, qb, c, m, z):
        ks = slice(c * _CK, (c + 1) * _CK)
        cols = slice(qb * _BQ, (qb + 1) * _BQ)
        p = jnp.exp2(bufs[qb % 2][ks, :] - m).astype(_BF16)
        pv = _mm(v_v[h + z, :, ks], p)
        o_v[h + z, :, cols] = pv if c == 0 else o_v[h + z, :, cols] + pv
        return pv

    def gate_up(i, z, j, kt):
        w = _unpack(jnp.concatenate(
            [r[64 * kt:64 * (kt + 1), _tile(2 * j, 2)] for r in (wg_v, wu_v)], axis=1))
        part = _mm(_unpack(xn_v[i + z, :, _tile(kt)]), w)
        gu = part if kt == 0 else gu_v[z] + part
        if kt < D // 128 - 1:
            gu_v[z] = gu
        else:
            g = 0.5 * gu[:, 0:256]
            hid = (g + g * jnp.tanh(g)) * gu[:, 256:512]
            hid_v[z, :, _tile(2 * j, 2)] = _pack(hid.astype(_BF16))
        return part

    def down(i, z, kt, nk, ct, nc):
        part = _mm(_unpack(hid_v[z, :, _tile(kt, nk)]),
                   _unpack(wd_v[64 * kt:64 * (kt + nk), _tile(ct, nc)]))
        cols = _tile(ct, nc)
        y_v[i + z, :, cols] = part if kt == 0 else y_v[i + z, :, cols] + part
        return part

    ffn = [(gate_up, (j, kt), kt == D // 128 - 1)
           for j in range(F // 256) for kt in range(D // 128)]
    for kt in range(F // 128):
        ffn.append((down, (kt, 1, 0, 4), False))
        if kt % 4 == 3:
            ffn.append((down, (kt - 3, 4, 4, 1), False))
    n_slot = 2 * n_q * n_ck
    ffn_at = {int(p * (n_slot - 1) / len(ffn)): f for p, f in enumerate(ffn)}

    bnd = [_NV + int(round(c * (S - _NV) / n_ck / 16)) * 16 for c in range(n_ck + 1)]
    segs = [(b, d0) for b in range(_NV // 8) for d0 in range(0, dh, _GD)]

    ops = []
    for slot in range(n_slot):
        ops += [("qk", slot, bnd[slot % n_ck + 1] - bnd[slot % n_ck]), ("pv", slot, _DP)]
        if slot in ffn_at:
            ops.append(("ffn", slot, rb))
    start = [0]
    for op in ops:
        start.append(start[-1] + op[2])
    free = [_VPU_RATE - 0.5] * (start[-1] + 2 * _LAT)
    for n, (kind, slot, dur) in enumerate(ops):
        if kind == "pv":
            t0, span, n_ops = start[max(n - 2, 0)], _EXP_SPAN, 160
        elif kind == "ffn" and ffn_at[slot][2]:
            t0, span, n_ops = start[n] + _LAT, dur, 176
        else:
            continue
        for t in range(t0, t0 + span):
            free[t] -= n_ops / span
    cum = [0.0]
    for f in free:
        cum.append(cum[-1] + max(f, 0.0))
    t_pop = {(kind, slot): start[n] + _LAT for n, (kind, slot, _) in enumerate(ops)}

    def due(kind, slot, r, last=False):
        if last:
            return len(segs)
        step = slot // n_ck
        lo = cum[t_pop["qk", step * n_ck]]
        hi = cum[t_pop.get(("qk", (step + 1) * n_ck), start[-1] + _LAT - 40)]
        now_ = cum[t_pop[kind, slot] + r + _LOOKAHEAD]
        return min(math.ceil(len(segs) * (now_ - lo) / (hi - lo)), len(segs))

    def head_step(i, par, carry):
        m1, m2 = carry
        h = 2 * i + par
        hp = jnp.maximum(h - 1, 0)
        hn = jnp.minimum(h + 1, _H - 1)
        never = lax.broadcasted_iota(_I32, (8, 128), 0) < (h >> 12)
        uid = [1000 * par]

        def zero():
            uid[0] += 1
            return (h + uid[0]) >> 12

        n_splat = 0
        for qb in range(n_q):
            old1 = (h, qb - 1) if qb >= 1 else (hp, qb - 1 + n_q)
            old2 = (h, qb - 2) if qb >= 2 else (hp, qb - 2 + n_q)
            cur = bufs[qb % 2]
            slot0 = (par * n_q + qb) * n_ck
            st = dict(pos=0, m=None)

            def vpu_scores(upto, anchor, qb=qb, cur=cur, st=st):
                while st["pos"] < upto:
                    b, d0 = segs[st["pos"]]
                    st["pos"] += 1
                    if d0 == 0:
                        st["z"] = zero()
                    for d in range(d0, d0 + _GD):
                        kb = kbs[par][st["z"], d, 8 * b:8 * b + 8, :]
                        if d == d0:
                            kb = jnp.where(never, anchor, kb)
                        term = jnp.concatenate([
                            kb * q_v[h + st["z"], d:d + 1, q:q + 128]
                            for q in range(qb * _BQ, (qb + 1) * _BQ, 128)], axis=1)
                        st["s"] = term if d == 0 else st["s"] + term
                    if d == dh - 1:
                        cur[8 * b:8 * b + 8, :] = st["s"]
                        st["m"] = jnp.maximum(st["m"], st["s"])

            for c in range(n_ck):
                slot = slot0 + c
                z = zero()
                kk = _unpack(k_v[h + z, bnd[c] // 2:bnd[c + 1] // 2, :])
                s = _mm(kk[:, 0:_DP], q_v[h + z, :, qb * _BQ:(qb + 1) * _BQ])
                if c < _LAG:
                    pv = pv_chunk(*old2, n_ck - _LAG + c, m2, z)
                else:
                    pv = pv_chunk(*old1, c - _LAG, m1, z)
                cur[bnd[c]:bnd[c + 1], :] = s
                for r in range(0, bnd[c + 1] - bnd[c], 8):
                    row = s[r:r + 8]
                    st["m"] = row if st["m"] is None else jnp.maximum(st["m"], row)
                    vpu_scores(due("qk", slot, r), row[:, 0:128])
                    frac = min((qb * n_ck + c + r / 96) / (n_q * n_ck - 3), 1)
                    while r in (16, 64) and n_splat < frac * len(splats):
                        splat_keys(hn + z, 1 - par, *splats[n_splat], lambda v: jnp.where(
                            never, pltpu.bitcast(row[:, 0:128], _I32), v))
                        n_splat += 1
                for r in range(0, _DP, 8):
                    last = c == n_ck - 1 and r == _DP - 8 and slot not in ffn_at
                    vpu_scores(due("pv", slot, r, last), pv[r:r + 8, 0:128])
                if slot in ffn_at:
                    fn, args, _ = ffn_at[slot]
                    part = fn(i, z, *args)
                    for r in range(0, rb, 8):
                        last = c == n_ck - 1 and r == rb - 8
                        vpu_scores(due("ffn", slot, r, last), part[r:r + 8, 0:128])
            assert st["pos"] == len(segs)
            m1, m2 = jnp.max(st["m"], axis=0, keepdims=True), m1
        assert n_splat == len(splats)
        return m1, m2

    zero_m = jnp.zeros((1, _BQ), _F32)
    m1, m2 = lax.fori_loop(
        0, _H // 2, lambda i, c: head_step(i, 1, head_step(i, 0, c)), (zero_m, zero_m))

    after = pacer()
    low = lax.broadcasted_iota(_I32, (8, 128), 0) < 4
    heads = [[] for _ in range(S // rb)]

    def normalize(j, h, pace):
        a = o_v[h, :, _tile(j)] * (1.0 / pace(o_v[h, _DP - 1:_DP, _tile(j)]))[0:1]
        b = o_v[h + 1, :, _tile(j)] * (1.0 / pace(o_v[h + 1, 0:1, _tile(j)]))[0:1]
        heads[j] += [a[0:16], jnp.where(low, a[16:24], b[0:8]), b[8:24]]
        if h + 2 == _H:
            xn_v[j] = _pack(jnp.concatenate(heads[j], axis=0).astype(_BF16).T)

    def norm_tasks(lo, hi):
        return [partial(normalize, j, h)
                for j in range(lo // rb, hi // rb) for h in range(0, _H, 2)]

    tail = [(n_q - 2, c, m2) for c in range(n_ck - _LAG, n_ck)]
    tail += [(n_q - 1, c, m1) for c in range(n_ck)]
    for task in norm_tasks(0, _O_CUT[1]):
        task(now)
    for i, (lo, hi) in enumerate(zip(_O_CUT[:-1], _O_CUT[1:])):
        blocks = slice(lo // rb, hi // rb)
        o = _unpack(xn_v[blocks].reshape((hi - lo) // 2, D))
        parts = []
        for t in range(D // 128):
            parts.append(_mm(o[:, _tile(t)], wo_v[_tile(t), 0:512]))
            for _ in range(min(2, len(tail)) if i >= 1 else 0):
                pv_chunk(_H - 1, *tail.pop(0), 0)
        tasks = norm_tasks(hi, _O_CUT[i + 2]) if hi < S else []
        assert not tasks or all(qb * _BQ >= _O_CUT[i + 2] for qb, _, _ in tail)
        n8 = (hi - lo) // 8
        for j, task in enumerate(tasks):
            t, r = divmod(j * 4 * n8 // len(tasks), n8)
            task(after(parts[t][8 * r:8 * r + 8, 0:128]))
        att = jnp.concatenate(
            [functools.reduce(jnp.add, parts), _mm(o, wo_v[:, 512:D])], axis=1)
        y = x_v[lo:hi, :].astype(_F32) + y_v[blocks].reshape(hi - lo, D) + att
        out_v[lo:hi, :] = y.astype(out_v.dtype)
        o_cp[i].start()
    for cp in o_cp:
        cp.wait()


@jax.jit
def pallas_parallel_sum__mha_block__swiglu_ffn__prompt_kernel(
    A_x: jax.Array,
    A_wqkv: jax.Array,
    A_wo: jax.Array,
    B_x: jax.Array,
    B_w_gate: jax.Array,
    B_w_up: jax.Array,
    B_w_down: jax.Array,
):
    del B_x
    B, S, D = A_x.shape
    F = B_w_gate.shape[1]
    assert (B, S, D, F) == (1, 2048, 640, 1536)
    n_it = _H // 2
    rb = S // n_it
    any_spec = pl.BlockSpec(memory_space=pl.ANY)
    out = pl.pallas_call(
        _kernel,
        out_shape=jax.ShapeDtypeStruct((S, D), _BF16),
        in_specs=[any_spec] * 6,
        out_specs=any_spec,
        scratch_shapes=[
            pltpu.VMEM((S, D), _BF16),
            pltpu.VMEM((n_it, rb // 2, D), _I32),
            pltpu.VMEM((D, S), _BF16),
            pltpu.VMEM((D, D), _BF16),
            pltpu.VMEM((D, D), _BF16),
            pltpu.VMEM((D, D), _BF16),
            pltpu.VMEM((D, D), _BF16),
            pltpu.VMEM((D // 2, F), _I32),
            pltpu.VMEM((D // 2, F), _I32),
            pltpu.VMEM((F // 2, D), _I32),
            pltpu.VMEM((D, D), _BF16),
            pltpu.VMEM((D, D), _BF16),
            pltpu.VMEM((S // 2, D), _I32),
            pltpu.VMEM((_H, _DP, S), _F32),
            pltpu.VMEM((_H, S // 2, 128), _I32),
            pltpu.VMEM((_H, _DP, S), _F32),
            pltpu.VMEM((_H, _DP, S), _F32),
            pltpu.VMEM((S, _BQ), _F32),
            pltpu.VMEM((S, _BQ), _F32),
            pltpu.VMEM((1, D // _H, _NV, 128), _F32),
            pltpu.VMEM((1, D // _H, _NV, 128), _F32),
            pltpu.VMEM((1, rb, 512), _F32),
            pltpu.VMEM((1, rb // 2, F), _I32),
            pltpu.VMEM((n_it, rb, D), _F32),
            pltpu.VMEM((S, D), _BF16),
            pltpu.VMEM((8, 128), _F32),
            pltpu.SemaphoreType.DMA((len(_X_CUT) - 1,)),
            pltpu.SemaphoreType.DMA((7,)),
            pltpu.SemaphoreType.DMA((len(_O_CUT) - 1,)),
        ],
        compiler_params=pltpu.CompilerParams(
            vmem_limit_bytes=110 * 1024 * 1024,
            flags={"XLA_TPU_EVENLY_DISTRIBUTE_CRITICAL_NODES": True},
        ),
        name="fused_mha_swiglu",
    )(*(a.astype(_BF16) for a in
        (A_x.reshape(S, D), A_wqkv, A_wo, B_w_gate, B_w_up, B_w_down)))
    return out.reshape(B, S, D).astype(A_x.dtype)
```

```python
import functools
import math

import jax
import jax.numpy as jnp
from jax import lax
import jax.experimental.pallas as pl
import jax.experimental.pallas.tpu as pltpu

_H = 32
_EPS = 1e-5
_BQ = 512
_CK = 128
_LAG = 2
_DP = 24
_NV = 256
_BK = 8
_GD = 4
_X_CUT = (0, 256, 512, 1280, 1536, 2048)
_O_CUT = (0, 128, 512, 1024, 1536, 1920, 2048)
_LAT, _EXP_SPAN, _LOOKAHEAD, _VPU_RATE = 125, 64, 32, 3.1

_F32 = jnp.float32
_BF16 = jnp.bfloat16
_I32 = jnp.int32


def _mm(a, b):
    return lax.dot_general(a, b, (((1,), (0,)), ((), ())), preferred_element_type=_F32)


def _pack(v):
    return pltpu.bitcast(v, _I32)


def _unpack(v):
    return pltpu.bitcast(v, _BF16)


def _tile(t, n=1):
    return slice(128 * t, 128 * (t + n))


def _hold(never, anchor, v):
    def tiled(t):
        t = jnp.concatenate([t] * (v.shape[1] // 128), axis=1)
        return jnp.concatenate([t] * pl.cdiv(v.shape[0], 8), axis=0)

    if anchor.dtype != v.dtype:
        anchor = pltpu.bitcast(anchor, v.dtype)
    return jnp.where(tiled(never) != 0, tiled(anchor), v)


def _mix(*lists):
    keyed = [((j + 0.5) / len(l), n, t) for n, l in enumerate(lists) for j, t in enumerate(l)]
    return [t for _, _, t in sorted(keyed, key=lambda e: e[:2])]


def _kernel(
    x_hbm, wqkv_hbm, wo_hbm, wg_hbm, wu_hbm, wd_hbm,
    out_hbm,
    x_v, xn_v, xnt_v, wq_v, wk_v, wv_v, wo_v, wg_v, wu_v, wd_v, wgu_v, wdp_v, wqt_v, wvt_v,
    kp_v, q_v, k_v, v_v, o_v, sa_v, sb_v, kb0_v, kb1_v, gu_v, hid_v, y_v, out_v, z_v,
    x_sem, w_sem, o_sem,
):
    S, D = x_v.shape
    F = wg_v.shape[1]
    dh = D // _H
    n_q = S // _BQ
    n_ck = S // _CK
    rb = y_v.shape[1]
    bufs = (sa_v, sb_v)
    kbs = (kb0_v, kb1_v)
    partial = functools.partial

    x_cp = [
        pltpu.make_async_copy(x_hbm.at[lo:hi], x_v.at[lo:hi], x_sem.at[i])
        for i, (lo, hi) in enumerate(zip(_X_CUT[:-1], _X_CUT[1:]))
    ]
    w_cp = [
        pltpu.make_async_copy(src, dst, w_sem.at[i])
        for i, (src, dst) in enumerate([
            (wqkv_hbm.at[:, D:2 * D], wk_v),
            (wqkv_hbm.at[:, 0:D], wq_v),
            (wqkv_hbm.at[:, 2 * D:3 * D], wv_v),
            (wg_hbm, wg_v),
            (wu_hbm, wu_v),
            (wd_hbm, wd_v),
            (wo_hbm, wo_v),
        ])
    ]
    o_cp = [
        pltpu.make_async_copy(out_v.at[lo:hi], out_hbm.at[lo:hi], o_sem.at[i])
        for i, (lo, hi) in enumerate(zip(_O_CUT[:-1], _O_CUT[1:]))
    ]

    def now(v):
        return v

    def pacer():
        never = z_v[...]
        return lambda anchor: partial(_hold, never, anchor)

    def layernorm(r0, pace):
        x = _unpack(pace(_pack(x_v[r0:r0 + 32, :]))).astype(_F32)
        xc = x - jnp.mean(x, axis=-1, keepdims=True)
        var = jnp.mean(xc * xc, axis=-1, keepdims=True)
        xn = (xc * lax.rsqrt(var + _EPS)).astype(_BF16)
        xn_v[r0 // rb, r0 % rb // 2:r0 % rb // 2 + 16, :] = _pack(xn)

    def transpose(src, dst, pace):
        dst[...] = _unpack(pace(_pack(src[...]))).T

    def repack(src, dst, pace):
        dst[...] = pace(_pack(src[...]))

    def spread_k(h, r0, pace):
        t, off = divmod(h * dh, 128)
        w = pace(kp_v[r0:r0 + 64, _tile(t)])
        if off + dh > 128:
            lane = lax.broadcasted_iota(_I32, w.shape, 1)
            w = jnp.where(lane >= 64, w, kp_v[r0:r0 + 64, _tile(t + 1)])
        k_v[h, r0:r0 + 64, :] = pltpu.roll(w, 128 - off, 1) if off else w

    def splat_keys(h, slot, d0, g, pace):
        kk = _unpack(pace(k_v[h, 8 * g:8 * g + 8, :])).astype(_F32)
        for d in range(d0, d0 + 5):
            kbs[slot][0, d, 16 * g:16 * g + 16, :] = jnp.broadcast_to(kk[:, d:d + 1], (16, 128))

    splats = [(d0, g) for d0 in range(0, dh, 5) for g in range(_NV // 16)]

    def dot_paced(lhs, rhs, tasks, after):
        nk = lhs.shape[1] // 128
        m8 = lhs.shape[0] // 8
        parts = [_mm(lhs[:, _tile(t)], rhs[_tile(t), :]) for t in range(nk)]
        for j, task in enumerate(tasks):
            t, r = divmod(int(j * (nk - 0.4) * m8 / len(tasks)), m8)
            task(after(parts[t][8 * r:8 * r + 8, 0:128]))
        return functools.reduce(jnp.add, parts)

    def project_k(r0, n, tasks, after):
        xn = _unpack(xn_v[r0 // rb:(r0 + n) // rb].reshape(n // 2, D))
        k = jnp.concatenate([
            dot_paced(xn, wk_v[:, 0:512], tasks, after), _mm(xn, wk_v[:, 512:D])], axis=1)
        kp_v[r0 // 2:(r0 + n) // 2, :] = _pack(k.astype(_BF16))

    sub = lax.broadcasted_iota(_I32, (8, _BQ), 0)

    def project_q(i, tasks, after):
        cols = slice(i * _BQ, (i + 1) * _BQ)
        qt = dot_paced(wqt_v[...], xnt_v[:, cols], tasks, after)
        qt = qt * (dh ** -0.5 * math.log2(math.e))
        for h in range(_H):
            base = h * dh // 8 * 8
            q3 = [qt[base + 8 * j:base + 8 * j + 8] for j in range(3)]
            if h % 2 == 0:
                q3[2] = jnp.where(sub < 4, q3[2], 0.0)
            else:
                q3 = [pltpu.roll(t, 4, 0) for t in q3] + [0.0]
                q3 = [jnp.where(sub < 4, q3[j], q3[j + 1]) for j in range(3)]
            q_v[h, :, cols] = jnp.concatenate(q3, axis=0)

    def project_v(i, tasks, after):
        cols = slice(i * _BQ, (i + 1) * _BQ)
        vt = dot_paced(wvt_v[...], xnt_v[:, cols], tasks, after)
        for h in range(_H):
            base = h * dh // 8 * 8
            if h % 2 == 0:
                v_v[h, 0:16, cols] = vt[base:base + 16]
                v_v[h, 16:24, cols] = jnp.where(sub == 7, 1.0, vt[base + 16:base + 24])
            else:
                v_v[h, 0:8, cols] = jnp.where(sub == 0, 1.0, vt[base:base + 8])
                v_v[h, 8:24, cols] = vt[base + 8:base + 24]

    def ln_tasks(lo, hi):
        return [partial(layernorm, r0) for r0 in range(lo, hi, 32)]

    def xt_tasks(lo, hi):
        return [partial(transpose, xn_v.at[j, :, _tile(t)], xnt_v.at[_tile(t), _tile(j)])
                for j in range(lo // rb, hi // rb) for t in range(D // 128)]

    def wt_tasks(src, dst):
        return [partial(transpose, src.at[_tile(r), _tile(c)], dst.at[_tile(c), _tile(r)])
                for r in range(D // 128) for c in range(D // 128)]

    def gu_tasks(n, src):
        return [partial(repack, src.at[r:r + 32, _tile(2 * j, 2)],
                        wgu_v.at[r // 2:r // 2 + 16, _tile(4 * j + 2 * n, 2)])
                for j in range(F // 256) for r in range(0, D, 32)]

    def ks_tasks(lo, hi):
        return [partial(spread_k, h, r0 // 2) for r0 in range(lo, hi, 128) for h in range(_H)]

    for cp in (x_cp[0], x_cp[1], w_cp[0]):
        cp.start()
    sa_v[S - _LAG * _CK:, :] = jnp.zeros((_LAG * _CK, _BQ), _F32)
    sb_v[...] = jnp.zeros(sb_v.shape, _F32)
    o_v[0, :, S - 2 * _BQ:S - _BQ] = jnp.zeros((_DP, _BQ), _F32)
    z_v[...] = jnp.zeros(z_v.shape, _F32)
    x_cp[0].wait()
    x_cp[2].start()
    for task in ln_tasks(0, 256):
        task(now)
    w_cp[0].wait()
    x_cp[3].start()
    x_cp[1].wait()
    after = pacer()
    project_k(0, 256, ln_tasks(256, 512), after)
    project_k(256, 128, [], after)
    x_cp[2].wait()
    for cp in (x_cp[4], w_cp[1], w_cp[2]):
        cp.start()
    x_cp[3].wait()
    after = pacer()
    project_k(384, 128, ln_tasks(512, 640), after)
    project_k(512, 128, ln_tasks(640, 896), after)
    project_k(640, 256, ln_tasks(896, 1280), after)
    project_k(896, 384, _mix(ln_tasks(1280, 1536), xt_tasks(0, 256)), after)
    w_cp[1].wait()
    w_cp[2].wait()
    for cp in w_cp[3:]:
        cp.start()
    x_cp[4].wait()
    after = pacer()
    project_k(1280, 256, _mix(wt_tasks(wq_v, wqt_v), xt_tasks(256, 512)), after)
    project_q(0, _mix(ln_tasks(1536, 1792), xt_tasks(512, 1024)), after)
    project_q(1, _mix(ln_tasks(1792, 2048), xt_tasks(1024, 1536)), after)
    project_k(1536, 512, _mix(xt_tasks(1536, 2048), ks_tasks(0, 256)), after)
    project_q(2, _mix(wt_tasks(wv_v, wvt_v), ks_tasks(256, 512)), after)
    project_q(3, ks_tasks(512, 896), after)
    project_v(0, [partial(splat_keys, 0, 0, *sp) for sp in splats], after)
    for cp in w_cp[3:]:
        cp.wait()
    after = pacer()
    project_v(1, _mix(ks_tasks(896, 1280), gu_tasks(0, wg_v)), after)
    project_v(2, _mix(ks_tasks(1280, 1664), gu_tasks(1, wu_v)), after)
    project_v(3, _mix(ks_tasks(1664, 2048), [
        partial(repack, wd_v.at[r:r + 16], wdp_v.at[r // 2:r // 2 + 8])
        for r in range(0, F, 16)]), after)

    def pv_chunk(h, qb, c, m, z):
        ks = slice(c * _CK, (c + 1) * _CK)
        cols = slice(qb * _BQ, (qb + 1) * _BQ)
        p = jnp.exp2(bufs[qb % 2][ks, :] - m).astype(_BF16)
        pv = _mm(v_v[h + z, :, ks], p)
        o_v[h + z, :, cols] = pv if c == 0 else o_v[h + z, :, cols] + pv
        return pv

    def gate_up(i, z, j, kt):
        w = _unpack(wgu_v[64 * kt:64 * (kt + 1), _tile(4 * j, 4)])
        part = _mm(_unpack(xn_v[i + z, :, _tile(kt)]), w)
        gu = part if kt == 0 else gu_v[z] + part
        if kt < D // 128 - 1:
            gu_v[z] = gu
        else:
            g = 0.5 * gu[:, 0:256]
            hid = (g + g * jnp.tanh(g)) * gu[:, 256:512]
            hid_v[z, :, _tile(2 * j, 2)] = _pack(hid.astype(_BF16))
        return part

    def down(i, z, kt, nk, ct, nc):
        cols = _tile(ct, nc)
        part = _mm(_unpack(hid_v[z, :, _tile(kt, nk)]),
                   _unpack(wdp_v[64 * kt:64 * (kt + nk), cols]))
        y_v[i + z, :, cols] = part if kt == 0 else y_v[i + z, :, cols] + part
        return part

    ffn = [(gate_up, (j, kt), kt == D // 128 - 1)
           for j in range(F // 256) for kt in range(D // 128)]
    for kt in range(F // 128):
        ffn.append((down, (kt, 1, 0, 4), False))
        if kt % 4 == 3:
            ffn.append((down, (kt - 3, 4, 4, 1), False))
    n_slot = 2 * n_q * n_ck
    ffn_at = {int(p * (n_slot - 1) / len(ffn)): f for p, f in enumerate(ffn)}

    bnd = [_NV + int(round(c * (S - _NV) / n_ck / 16)) * 16 for c in range(n_ck + 1)]
    segs = [(b, d0) for b in range(0, _NV, _BK) for d0 in range(0, dh, _GD)]

    ops = []
    for slot in range(n_slot):
        ops += [("qk", slot, bnd[slot % n_ck + 1] - bnd[slot % n_ck]), ("pv", slot, _DP)]
        if slot in ffn_at:
            ops.append(("ffn", slot, rb))
    start = [0]
    for op in ops:
        start.append(start[-1] + op[2])
    free = [_VPU_RATE - 0.5] * (start[-1] + 2 * _LAT)
    for n, (kind, slot, dur) in enumerate(ops):
        if kind == "pv":
            t0, span, n_ops = start[max(n - 2, 0)], _EXP_SPAN, 160
        elif kind == "ffn" and ffn_at[slot][2]:
            t0, span, n_ops = start[n] + _LAT, dur, 176
        else:
            continue
        for t in range(t0, t0 + span):
            free[t] -= n_ops / span
    cum = [0.0]
    for f in free:
        cum.append(cum[-1] + max(f, 0.0))
    t_pop = {(kind, slot): start[n] + _LAT for n, (kind, slot, _) in enumerate(ops)}

    def due(kind, slot, r, last=False):
        if last:
            return len(segs)
        step = slot // n_ck
        lo = cum[t_pop["qk", step * n_ck]]
        hi = cum[t_pop.get(("qk", (step + 1) * n_ck), start[-1] + _LAT - 40)]
        now_ = cum[t_pop[kind, slot] + r + _LOOKAHEAD]
        return min(math.ceil(len(segs) * (now_ - lo) / (hi - lo)), len(segs))

    def head_step(i, par, carry):
        m1, m2 = carry
        h = 2 * i + par
        hp = jnp.maximum(h - 1, 0)
        hn = jnp.minimum(h + 1, _H - 1)
        never = z_v[...]
        uid = [1000 * par]

        def zero():
            uid[0] += 1
            return (h + uid[0]) >> 12

        n_splat = 0
        for qb in range(n_q):
            old1 = (h, qb - 1) if qb >= 1 else (hp, qb - 1 + n_q)
            old2 = (h, qb - 2) if qb >= 2 else (hp, qb - 2 + n_q)
            cur = bufs[qb % 2]
            slot0 = (par * n_q + qb) * n_ck
            st = dict(pos=0, m=None)

            def vpu_scores(upto, anchor, qb=qb, cur=cur, st=st):
                while st["pos"] < upto:
                    b, d0 = segs[st["pos"]]
                    st["pos"] += 1
                    if d0 == 0:
                        st["z"] = zero()
                        st["h"] = h + st["z"]
                    for d in range(d0, d0 + _GD):
                        kb = kbs[par][st["z"], d, b:b + _BK, :]
                        if d == d0:
                            kb = _hold(never, anchor, kb)
                        term = jnp.concatenate([
                            kb * q_v[st["h"], d:d + 1, q:q + 128]
                            for q in range(qb * _BQ, (qb + 1) * _BQ, 128)], axis=1)
                        st["s"] = term if d == 0 else st["s"] + term
                    if d == dh - 1:
                        cur[b:b + _BK, :] = st["s"]
                        for r in range(0, _BK, 8):
                            st["m"] = jnp.maximum(st["m"], st["s"][r:r + 8])

            for c in range(n_ck):
                slot = slot0 + c
                z = zero()
                kk = _unpack(k_v[h + z, bnd[c] // 2:bnd[c + 1] // 2, :])
                s = _mm(kk[:, 0:_DP], q_v[h + z, :, qb * _BQ:(qb + 1) * _BQ])
                if c < _LAG:
                    pv = pv_chunk(*old2, n_ck - _LAG + c, m2, z)
                else:
                    pv = pv_chunk(*old1, c - _LAG, m1, z)
                cur[bnd[c]:bnd[c + 1], :] = s
                for r in range(0, bnd[c + 1] - bnd[c], 8):
                    row = s[r:r + 8]
                    st["m"] = row if st["m"] is None else jnp.maximum(st["m"], row)
                    vpu_scores(due("qk", slot, r), row[:, 0:128])
                    frac = min((qb * n_ck + c + r / 96) / (n_q * n_ck - 3), 1)
                    while r in (16, 64) and n_splat < frac * len(splats):
                        splat_keys(hn + z, 1 - par, *splats[n_splat], partial(_hold, never, row[:, 0:128]))
                        n_splat += 1
                for r in range(0, _DP, 8):
                    last = c == n_ck - 1 and r == _DP - 8 and slot not in ffn_at
                    vpu_scores(due("pv", slot, r, last), pv[r:r + 8, 0:128])
                if slot in ffn_at:
                    fn, args, _ = ffn_at[slot]
                    part = fn(i, z, *args)
                    for r in range(0, rb, 8):
                        last = c == n_ck - 1 and r == rb - 8
                        vpu_scores(due("ffn", slot, r, last), part[r:r + 8, 0:128])
            assert st["pos"] == len(segs)
            m1, m2 = jnp.max(st["m"], axis=0, keepdims=True), m1
        assert n_splat == len(splats)
        return m1, m2

    zero_m = jnp.zeros((1, _BQ), _F32)
    m1, m2 = lax.fori_loop(
        0, _H // 2, lambda i, c: head_step(i, 1, head_step(i, 0, c)), (zero_m, zero_m))

    after = pacer()
    low = lax.broadcasted_iota(_I32, (8, 128), 0) < 4
    heads = [[] for _ in range(S // rb)]

    def normalize(j, h, pace):
        a = o_v[h, :, _tile(j)] * (1.0 / pace(o_v[h, _DP - 1:_DP, _tile(j)]))[0:1]
        b = o_v[h + 1, :, _tile(j)] * (1.0 / pace(o_v[h + 1, 0:1, _tile(j)]))[0:1]
        heads[j] += [a[0:16], jnp.where(low, a[16:24], b[0:8]), b[8:24]]
        if h + 2 == _H:
            xn_v[j] = _pack(jnp.concatenate(heads[j], axis=0).astype(_BF16).T)

    def norm_tasks(lo, hi):
        return [partial(normalize, j, h)
                for j in range(lo // rb, hi // rb) for h in range(0, _H, 2)]

    tail = [(n_q - 2, c, m2) for c in range(n_ck - _LAG, n_ck)]
    tail += [(n_q - 1, c, m1) for c in range(n_ck)]
    for task in norm_tasks(0, _O_CUT[1]):
        task(now)
    for i, (lo, hi) in enumerate(zip(_O_CUT[:-1], _O_CUT[1:])):
        blocks = slice(lo // rb, hi // rb)
        o = _unpack(xn_v[blocks].reshape((hi - lo) // 2, D))
        parts = []
        for t in range(D // 128):
            parts.append(_mm(o[:, _tile(t)], wo_v[_tile(t), 0:512]))
            for _ in range(min(2, len(tail)) if i >= 1 else 0):
                pv_chunk(_H - 1, *tail.pop(0), 0)
        tasks = norm_tasks(hi, _O_CUT[i + 2]) if hi < S else []
        assert not tasks or all(qb * _BQ >= _O_CUT[i + 2] for qb, _, _ in tail)
        n8 = (hi - lo) // 8
        for j, task in enumerate(tasks):
            t, r = divmod(j * 4 * n8 // len(tasks), n8)
            task(after(parts[t][8 * r:8 * r + 8, 0:128]))
        att = jnp.concatenate(
            [functools.reduce(jnp.add, parts), _mm(o, wo_v[:, 512:D])], axis=1)
        y = x_v[lo:hi, :].astype(_F32) + y_v[blocks].reshape(hi - lo, D) + att
        out_v[lo:hi, :] = y.astype(out_v.dtype)
        o_cp[i].start()
    for cp in o_cp:
        cp.wait()


@jax.jit
def pallas_parallel_sum__mha_block__swiglu_ffn__prompt_kernel(
    A_x: jax.Array,
    A_wqkv: jax.Array,
    A_wo: jax.Array,
    B_x: jax.Array,
    B_w_gate: jax.Array,
    B_w_up: jax.Array,
    B_w_down: jax.Array,
):
    del B_x
    B, S, D = A_x.shape
    F = B_w_gate.shape[1]
    assert (B, S, D, F) == (1, 2048, 640, 1536)
    n_it = _H // 2
    rb = S // n_it
    any_spec = pl.BlockSpec(memory_space=pl.ANY)
    out = pl.pallas_call(
        _kernel,
        out_shape=jax.ShapeDtypeStruct((S, D), _BF16),
        in_specs=[any_spec] * 6,
        out_specs=any_spec,
        scratch_shapes=[
            pltpu.VMEM((S, D), _BF16),
            pltpu.VMEM((n_it, rb // 2, D), _I32),
            pltpu.VMEM((D, S), _BF16),
            pltpu.VMEM((D, D), _BF16),
            pltpu.VMEM((D, D), _BF16),
            pltpu.VMEM((D, D), _BF16),
            pltpu.VMEM((D, D), _BF16),
            pltpu.VMEM((D, F), _BF16),
            pltpu.VMEM((D, F), _BF16),
            pltpu.VMEM((F, D), _BF16),
            pltpu.VMEM((D // 2, 2 * F), _I32),
            pltpu.VMEM((F // 2, D), _I32),
            pltpu.VMEM((D, D), _BF16),
            pltpu.VMEM((D, D), _BF16),
            pltpu.VMEM((S // 2, D), _I32),
            pltpu.VMEM((_H, _DP, S), _F32),
            pltpu.VMEM((_H, S // 2, 128), _I32),
            pltpu.VMEM((_H, _DP, S), _F32),
            pltpu.VMEM((_H, _DP, S), _F32),
            pltpu.VMEM((S, _BQ), _F32),
            pltpu.VMEM((S, _BQ), _F32),
            pltpu.VMEM((1, D // _H, _NV, 128), _F32),
            pltpu.VMEM((1, D // _H, _NV, 128), _F32),
            pltpu.VMEM((1, rb, 512), _F32),
            pltpu.VMEM((1, rb // 2, F), _I32),
            pltpu.VMEM((n_it, rb, D), _F32),
            pltpu.VMEM((S, D), _BF16),
            pltpu.VMEM((8, 128), _F32),
            pltpu.SemaphoreType.DMA((len(_X_CUT) - 1,)),
            pltpu.SemaphoreType.DMA((7,)),
            pltpu.SemaphoreType.DMA((len(_O_CUT) - 1,)),
        ],
        compiler_params=pltpu.CompilerParams(
            vmem_limit_bytes=110 * 1024 * 1024,
            flags={"XLA_TPU_EVENLY_DISTRIBUTE_CRITICAL_NODES": True},
        ),
        name="fused_mha_swiglu",
    )(*(a.astype(_BF16) for a in
        (A_x.reshape(S, D), A_wqkv, A_wo, B_w_gate, B_w_up, B_w_down)))
    return out.reshape(B, S, D).astype(A_x.dtype)
```
